```python
import os as _os
_os.environ.setdefault("JAX_PLATFORMS", "cpu")
import jax
import jax.numpy as jnp

def _softmax(x, axis=-1):
    return jax.nn.softmax(x, axis=axis)
def _gelu(x):
    return jax.nn.gelu(x, approximate=True)
def _silu(x):
    return jax.nn.silu(x)
def _sigmoid(x):
    return jax.nn.sigmoid(x)
def _layernorm(x, axis=-1, eps=1e-5):
    m = jnp.mean(x, axis=axis, keepdims=True)
    v = jnp.var(x, axis=axis, keepdims=True)
    return (x - m) / jnp.sqrt(v + eps)
def _scatter_add(tgt, idx, src, axis=0):
    return tgt.at[idx].add(src)
def _segment_sum(src, seg, n):
    return jax.ops.segment_sum(src, seg, n)
class _Rng:
    def __init__(self, key):
        self._k = key
    def _next(self):
        self._k, sub = jax.random.split(self._k)
        return sub
    def normal(self, shape):
        return jax.random.normal(self._next(), shape, dtype=jnp.bfloat16)
    def randint(self, lo, hi, shape):
        return jax.random.randint(self._next(), shape, lo, hi, dtype=jnp.int32)
    def uniform(self, shape, lo=0.0, hi=1.0):
        return jax.random.uniform(self._next(), shape, jnp.bfloat16, lo, hi)
    def permutation(self, n):
        return jax.random.permutation(self._next(), n)


kernel_name = 'standalone__moe_arch_mod__prompt'

def setup_inputs():
    _rng = _Rng(jax.random.key(int.from_bytes(__import__("os").urandom(4), "little")))
    _w = (lambda a: (lambda t: t.astype(jnp.bfloat16) if jnp.issubdtype(t.dtype, jnp.floating) else t)(jnp.asarray(a)))
    B, S, D, F, C = 1, 2048, 576, 4608, 8
    return {
        "x": _w((lambda *s: _rng.normal(s) * 0.1)(B, S, D)),
        "w_r": _w((lambda *s: _rng.normal(s) * 0.1)(D)),
        "w_gate": _w((lambda *s: _rng.normal(s) * 0.1)(D, F)),
        "w_up": _w((lambda *s: _rng.normal(s) * 0.1)(D, F)),
        "w_down": _w((lambda *s: _rng.normal(s) * 0.1)(F, D)),
    }

def reference(x, w_r, w_gate, w_up, w_down):
    B, S, D = x.shape
    C = 8
    r = x @ w_r
    idx = jnp.argsort(-r, axis=-1)[:, :C]
    idx_e = jnp.repeat(idx.reshape(B, C, 1), D, axis=2)
    x_sel = jnp.take_along_axis(x, idx_e, axis=1)
    g = _silu(x_sel @ w_gate)
    u = x_sel @ w_up
    y = (g * u) @ w_down
    r_sel = _sigmoid(jnp.take_along_axis(r, idx, axis=1))
    y = y * r_sel.reshape(B, C, 1)
    b_off = (jnp.arange(B) * S).reshape(B, 1)
    flat_idx = (idx + b_off).reshape(B * C)
    zero = (x * 0.0).reshape(B * S, D)
    upd = _scatter_add(zero, flat_idx, y.reshape(B * C, D), axis=0)
    return x + upd.reshape(B, S, D)
```

```python
import jax
import jax.numpy as jnp
from jax import lax
import jax.experimental.pallas as pl
import jax.experimental.pallas.tpu as pltpu

_C = 8
_LANES = 128
_NT = (((1,), (1,)), ((), ()))
_TN = (((0,), (0,)), ((), ()))
_INT_MIN = -(2**31)
_BOUNDS = (0, 128, 256, 384, 448, 544, 576)
_EARLY_STRIPS = 7


def _bf16_round(v):
    return v.astype(jnp.bfloat16).astype(jnp.float32)


def _kernel(x_hbm, wr_hbm, wg_hbm, wu_hbm, wd_hbm, o_hbm,
            xb, wrb, gb, ub, db, ob, rsem, wsem):
    D, S = xb.shape
    chunks = list(zip(_BOUNDS[:-1], _BOUNDS[1:]))
    r1, r2 = _BOUNDS[-3], _BOUNDS[-2]
    n_strips = S // _LANES
    strips = [i + j for j in range(4) for i in range(0, n_strips, 4)]

    c_x = pltpu.make_async_copy(x_hbm, xb, rsem.at[0])
    c_wr = pltpu.make_async_copy(wr_hbm, wrb, rsem.at[1])
    c_g = pltpu.make_async_copy(wg_hbm, gb, rsem.at[2])
    c_u = pltpu.make_async_copy(wu_hbm, ub, rsem.at[3])
    c_d = [
        pltpu.make_async_copy(wd_hbm.at[pl.ds(lo, hi - lo)],
                              db.at[pl.ds(lo, hi - lo)], rsem.at[4 + i])
        for i, (lo, hi) in enumerate(chunks)
    ]
    for c in (c_x, c_wr, c_g, c_u, *c_d):
        c.start()

    def write(lo, hi, c0, c1):
        sl = (pl.ds(lo, hi - lo), pl.ds(c0, c1 - c0))
        pltpu.make_async_copy(ob.at[sl], o_hbm.at[sl], wsem.at[0]).start()

    c_x.wait()
    c_wr.wait()
    xT = xb[...]
    wr8 = jnp.broadcast_to(wrb[...].reshape(1, D), (_C, D))
    r = _bf16_round(jnp.dot(wr8, xT, preferred_element_type=jnp.float32))

    bits = pltpu.bitcast(jnp.where(r == 0.0, 0.0, r), jnp.int32)
    mono = jnp.where(bits >= 0, bits, bits ^ 0x7FFFFFFF)
    mono = jnp.where(r != r, _INT_MIN, mono & -65536)
    lane = lax.broadcasted_iota(jnp.int32, (_C, S), 1)
    row = lax.broadcasted_iota(jnp.int32, (_C, S), 0)
    key = mono | (65535 - lane)
    sel = jnp.zeros((_C, S), jnp.float32)
    for c in range(_C):
        hit = key == jnp.max(key, axis=1, keepdims=True)
        sel = jnp.where(hit & (row == c), 1.0, sel)
        key = jnp.where(hit, _INT_MIN, key)
    onehot = sel.astype(jnp.bfloat16)
    r_sel = jnp.sum(jnp.where(sel > 0, r, 0.0), axis=1, keepdims=True)
    gate = _bf16_round(jax.nn.sigmoid(r_sel))

    x_sel = lax.dot_general(onehot, xT, _NT,
                            preferred_element_type=jnp.float32).astype(jnp.bfloat16)
    c_g.wait()
    g = _bf16_round(jnp.dot(x_sel, gb[...], preferred_element_type=jnp.float32))
    g = _bf16_round(g * jax.nn.sigmoid(g))
    c_u.wait()
    u = _bf16_round(jnp.dot(x_sel, ub[...], preferred_element_type=jnp.float32))
    h = (g * u).astype(jnp.bfloat16)

    for i, (lo, hi) in enumerate(chunks):
        c_d[i].wait()
        if lo == r1:
            for j in strips[:_EARLY_STRIPS]:
                write(0, r1, j * _LANES, (j + 1) * _LANES)
        y = _bf16_round(lax.dot_general(h, db[lo:hi, :], _NT,
                                        preferred_element_type=jnp.float32))
        y = (y * gate).astype(jnp.bfloat16)
        upd = lax.dot_general(y, onehot, _TN, preferred_element_type=jnp.float32)
        xc = xb[lo:hi, :].astype(jnp.float32)
        ob[lo:hi, :] = (xc + (xc * 0.0 + upd)).astype(ob.dtype)
        if lo == r1:
            for j in strips[_EARLY_STRIPS:]:
                write(0, r2, j * _LANES, (j + 1) * _LANES)
            for j in strips[:_EARLY_STRIPS]:
                write(r1, r2, j * _LANES, (j + 1) * _LANES)
    write(r2, D, 0, S)
    pltpu.make_async_copy(ob, o_hbm, wsem.at[0]).wait()


@jax.jit
def pallas_standalone__moe_arch_mod__prompt_kernel(
    x: jax.Array,
    w_r: jax.Array,
    w_gate: jax.Array,
    w_up: jax.Array,
    w_down: jax.Array,
):
    B, S, D = x.shape
    F = w_gate.shape[1]
    assert B == 1 and D == _BOUNDS[-1] and S % (4 * _LANES) == 0
    dt = x.dtype
    out_t = pl.pallas_call(
        _kernel,
        out_shape=jax.ShapeDtypeStruct((D, S), dt),
        in_specs=[pl.BlockSpec(memory_space=pl.ANY)] * 5,
        out_specs=pl.BlockSpec(memory_space=pl.ANY),
        scratch_shapes=[
            pltpu.VMEM((D, S), dt),
            pltpu.VMEM((D,), dt),
            pltpu.VMEM((D, F), dt),
            pltpu.VMEM((D, F), dt),
            pltpu.VMEM((D, F), dt),
            pltpu.VMEM((D, S), dt),
            pltpu.SemaphoreType.DMA((3 + len(_BOUNDS),)),
            pltpu.SemaphoreType.DMA((1,)),
        ],
        compiler_params=pltpu.CompilerParams(
            vmem_limit_bytes=64 * 1024 * 1024,
            disable_semaphore_checks=True,
        ),
    )(jnp.transpose(x.reshape(S, D)), w_r, w_gate, w_up, jnp.transpose(w_down))
    return jnp.transpose(out_t).reshape(B, S, D)
```

```python
import jax
import jax.numpy as jnp
from jax import lax
import jax.experimental.pallas as pl
import jax.experimental.pallas.tpu as pltpu

_C = 8
_LANES = 128
_NT = (((1,), (1,)), ((), ()))
_TN = (((0,), (0,)), ((), ()))
_INT_MIN = -(2**31)
_BOUNDS = (0, 128, 256, 368, 448, 536, 576)
_CUE_COLS = 2048
_EARLY_STRIPS = 7


def _bf16_round(v):
    return v.astype(jnp.bfloat16).astype(jnp.float32)


def _kernel(x_hbm, wr_hbm, wg_hbm, wu_hbm, wd_hbm, o_hbm,
            xb, wrb, gb, ub, db, ob, rsem, wsem):
    D, S = xb.shape
    F = db.shape[1]
    chunks = list(zip(_BOUNDS[:-1], _BOUNDS[1:]))
    r1, r2 = _BOUNDS[-3], _BOUNDS[-2]
    n_strips = S // _LANES
    strips = [i + j for j in range(4) for i in range(0, n_strips, 4)]
    early, late = strips[:_EARLY_STRIPS], strips[_EARLY_STRIPS:]
    assert len(late) >= len(early)

    c_x = pltpu.make_async_copy(x_hbm, xb, rsem.at[0])
    c_wr = pltpu.make_async_copy(wr_hbm, wrb, rsem.at[1])
    c_g = pltpu.make_async_copy(wg_hbm, gb, rsem.at[2])
    c_u = pltpu.make_async_copy(wu_hbm, ub, rsem.at[3])

    def read_d(lo, hi, c0, c1, k):
        sl = (pl.ds(lo, hi - lo), pl.ds(c0, c1 - c0))
        return pltpu.make_async_copy(wd_hbm.at[sl], db.at[sl], rsem.at[4 + k])

    n = len(chunks)
    c_d = [[read_d(lo, hi, 0, F, i)] for i, (lo, hi) in enumerate(chunks[:-1])]
    c_d[-1].append(read_d(r2, r2 + 8, 0, _CUE_COLS, n - 2))
    c_d.append([read_d(r2, r2 + 8, _CUE_COLS, F, n - 1),
                read_d(r2 + 8, D, 0, F, n - 1)])
    for c in (c_x, c_wr, c_g, c_u, *[c for cs in c_d for c in cs]):
        c.start()

    def write(lo, hi, j):
        sl = (pl.ds(lo, hi - lo), pl.ds(j * _LANES, _LANES))
        pltpu.make_async_copy(ob.at[sl], o_hbm.at[sl], wsem.at[0]).start()

    c_x.wait()
    c_wr.wait()
    xT = xb[...]
    wr8 = jnp.broadcast_to(wrb[...].reshape(1, D), (_C, D))
    r = _bf16_round(jnp.dot(wr8, xT, preferred_element_type=jnp.float32))

    bits = pltpu.bitcast(jnp.where(r == 0.0, 0.0, r), jnp.int32)
    mono = jnp.where(bits >= 0, bits, bits ^ 0x7FFFFFFF)
    mono = jnp.where(r != r, _INT_MIN, mono & -65536)
    lane = lax.broadcasted_iota(jnp.int32, (_C, S), 1)
    row = lax.broadcasted_iota(jnp.int32, (_C, S), 0)
    key = mono | (65535 - lane)
    sel = jnp.zeros((_C, S), jnp.float32)
    for c in range(_C):
        hit = key == jnp.max(key, axis=1, keepdims=True)
        sel = jnp.where(hit & (row == c), 1.0, sel)
        key = jnp.where(hit, _INT_MIN, key)
    onehot = sel.astype(jnp.bfloat16)
    r_sel = jnp.sum(jnp.where(sel > 0, r, 0.0), axis=1, keepdims=True)
    gate = _bf16_round(jax.nn.sigmoid(r_sel))

    x_sel = lax.dot_general(onehot, xT, _NT,
                            preferred_element_type=jnp.float32).astype(jnp.bfloat16)
    c_g.wait()
    g = _bf16_round(jnp.dot(x_sel, gb[...], preferred_element_type=jnp.float32))
    g = _bf16_round(g * jax.nn.sigmoid(g))
    c_u.wait()
    u = _bf16_round(jnp.dot(x_sel, ub[...], preferred_element_type=jnp.float32))
    h = (g * u).astype(jnp.bfloat16)

    for i, (lo, hi) in enumerate(chunks):
        for c in c_d[i]:
            c.wait()
        if lo == r1:
            for j in early:
                write(0, r1, j)
        y = _bf16_round(lax.dot_general(h, db[lo:hi, :], _NT,
                                        preferred_element_type=jnp.float32))
        y = (y * gate).astype(jnp.bfloat16)
        upd = lax.dot_general(y, onehot, _TN, preferred_element_type=jnp.float32)
        xc = xb[lo:hi, :].astype(jnp.float32)
        ob[lo:hi, :] = (xc + (xc * 0.0 + upd)).astype(ob.dtype)
        if lo == r1:
            for t, j in enumerate(late):
                write(0, r2, j)
                if t < len(early):
                    write(r1, r2, early[t])
    for j in strips:
        write(r2, D, j)
    pltpu.make_async_copy(ob, o_hbm, wsem.at[0]).wait()


@jax.jit
def pallas_standalone__moe_arch_mod__prompt_kernel(
    x: jax.Array,
    w_r: jax.Array,
    w_gate: jax.Array,
    w_up: jax.Array,
    w_down: jax.Array,
):
    B, S, D = x.shape
    F = w_gate.shape[1]
    assert B == 1 and D == _BOUNDS[-1] and S % (4 * _LANES) == 0
    dt = x.dtype
    out_t = pl.pallas_call(
        _kernel,
        out_shape=jax.ShapeDtypeStruct((D, S), dt),
        in_specs=[pl.BlockSpec(memory_space=pl.ANY)] * 5,
        out_specs=pl.BlockSpec(memory_space=pl.ANY),
        scratch_shapes=[
            pltpu.VMEM((D, S), dt),
            pltpu.VMEM((D,), dt),
            pltpu.VMEM((D, F), dt),
            pltpu.VMEM((D, F), dt),
            pltpu.VMEM((D, F), dt),
            pltpu.VMEM((D, S), dt),
            pltpu.SemaphoreType.DMA((3 + len(_BOUNDS),)),
            pltpu.SemaphoreType.DMA((1,)),
        ],
        compiler_params=pltpu.CompilerParams(
            vmem_limit_bytes=64 * 1024 * 1024,
            disable_semaphore_checks=True,
        ),
    )(jnp.transpose(x.reshape(S, D)), w_r, w_gate, w_up, jnp.transpose(w_down))
    return jnp.transpose(out_t).reshape(B, S, D)
```

```python
import jax
import jax.numpy as jnp
from jax import lax
import jax.experimental.pallas as pl
import jax.experimental.pallas.tpu as pltpu

_C = 8
_LANES = 128
_NT = (((1,), (1,)), ((), ()))
_TN = (((0,), (0,)), ((), ()))
_INT_MIN = -(2**31)
_BOUNDS = (0, 80, 208, 320, 400, 464, 528, 576)
_CUE_ROWS, _CUE_COLS = 16, 3456
_EARLY_STRIPS = 6


def _bf16_round(v):
    return v.astype(jnp.bfloat16).astype(jnp.float32)


def _sigmoid_bf16(v):
    return _bf16_round(1.0 / _bf16_round(1.0 + _bf16_round(jnp.exp(-v))))


def _kernel(x_hbm, wr_hbm, wg_hbm, wu_hbm, wd_hbm, o_hbm,
            xb, wrb, gb, ub, db, ob, rsem, wsem):
    D, S = xb.shape
    F = db.shape[1]
    chunks = list(zip(_BOUNDS[:-1], _BOUNDS[1:]))
    r1, r2 = _BOUNDS[-3], _BOUNDS[-2]
    n_strips = S // _LANES
    strips = [i + j for j in range(4) for i in range(0, n_strips, 4)]
    early, late = strips[:_EARLY_STRIPS], strips[_EARLY_STRIPS:]
    assert len(late) >= len(early)

    c_x = pltpu.make_async_copy(x_hbm, xb, rsem.at[0])
    c_wr = pltpu.make_async_copy(wr_hbm, wrb, rsem.at[1])
    c_g = pltpu.make_async_copy(wg_hbm, gb, rsem.at[2])
    c_u = pltpu.make_async_copy(wu_hbm, ub, rsem.at[3])

    def read_d(lo, hi, c0, c1, k):
        sl = (pl.ds(lo, hi - lo), pl.ds(c0, c1 - c0))
        return pltpu.make_async_copy(wd_hbm.at[sl], db.at[sl], rsem.at[4 + k])

    n = len(chunks)
    c_d = [[read_d(lo, hi, 0, F, i)] for i, (lo, hi) in enumerate(chunks[:-1])]
    c_d[-1].append(read_d(r2, r2 + _CUE_ROWS, 0, _CUE_COLS, n - 2))
    c_d.append([read_d(r2, r2 + _CUE_ROWS, _CUE_COLS, F, n - 1),
                read_d(r2 + _CUE_ROWS, D, 0, F, n - 1)])
    for c in (c_x, c_wr, c_g, c_u, *[c for cs in c_d for c in cs]):
        c.start()

    def write(lo, hi, j):
        sl = (pl.ds(lo, hi - lo), pl.ds(j * _LANES, _LANES))
        pltpu.make_async_copy(ob.at[sl], o_hbm.at[sl], wsem.at[0]).start()

    c_x.wait()
    c_wr.wait()
    xT = xb[...]
    wr8 = jnp.broadcast_to(wrb[...].reshape(1, D), (_C, D))
    r = _bf16_round(jnp.dot(wr8, xT, preferred_element_type=jnp.float32))

    bits = pltpu.bitcast(jnp.where(r == 0.0, 0.0, r), jnp.int32)
    mono = jnp.where(bits >= 0, bits, bits ^ 0x7FFFFFFF)
    mono = jnp.where(r != r, _INT_MIN, mono & -65536)
    lane = lax.broadcasted_iota(jnp.int32, (_C, S), 1)
    row = lax.broadcasted_iota(jnp.int32, (_C, S), 0)
    key = mono | (65535 - lane)
    sel = jnp.zeros((_C, S), jnp.float32)
    for c in range(_C):
        hit = key == jnp.max(key, axis=1, keepdims=True)
        sel = jnp.where(hit & (row == c), 1.0, sel)
        key = jnp.where(hit, _INT_MIN, key)
    onehot = sel.astype(jnp.bfloat16)
    r_sel = jnp.sum(jnp.where(sel > 0, r, 0.0), axis=1, keepdims=True)
    gate = _sigmoid_bf16(r_sel)

    x_sel = lax.dot_general(onehot, xT, _NT,
                            preferred_element_type=jnp.float32).astype(jnp.bfloat16)
    c_g.wait()
    g = _bf16_round(jnp.dot(x_sel, gb[...], preferred_element_type=jnp.float32))
    g = _bf16_round(g * _sigmoid_bf16(g))
    c_u.wait()
    u = _bf16_round(jnp.dot(x_sel, ub[...], preferred_element_type=jnp.float32))
    h = (g * u).astype(jnp.bfloat16)

    for i, (lo, hi) in enumerate(chunks):
        for c in c_d[i]:
            c.wait()
        if lo == r1:
            for j in early:
                write(0, r1, j)
        y = _bf16_round(lax.dot_general(h, db[lo:hi, :], _NT,
                                        preferred_element_type=jnp.float32))
        y = (y * gate).astype(jnp.bfloat16)
        upd = lax.dot_general(y, onehot, _TN, preferred_element_type=jnp.float32)
        xc = xb[lo:hi, :].astype(jnp.float32)
        ob[lo:hi, :] = (xc + (xc * 0.0 + upd)).astype(ob.dtype)
        if lo == r1:
            for t, j in enumerate(late):
                write(0, r2, j)
                if t < len(early):
                    write(r1, r2, early[t])
    for j in strips:
        write(r2, D, j)
    pltpu.make_async_copy(ob, o_hbm, wsem.at[0]).wait()


@jax.jit
def pallas_standalone__moe_arch_mod__prompt_kernel(
    x: jax.Array,
    w_r: jax.Array,
    w_gate: jax.Array,
    w_up: jax.Array,
    w_down: jax.Array,
):
    B, S, D = x.shape
    F = w_gate.shape[1]
    assert B == 1 and D == _BOUNDS[-1] and S % (4 * _LANES) == 0
    dt = x.dtype
    out_t = pl.pallas_call(
        _kernel,
        out_shape=jax.ShapeDtypeStruct((D, S), dt),
        in_specs=[pl.BlockSpec(memory_space=pl.ANY)] * 5,
        out_specs=pl.BlockSpec(memory_space=pl.ANY),
        scratch_shapes=[
            pltpu.VMEM((D, S), dt),
            pltpu.VMEM((D,), dt),
            pltpu.VMEM((D, F), dt),
            pltpu.VMEM((D, F), dt),
            pltpu.VMEM((D, F), dt),
            pltpu.VMEM((D, S), dt),
            pltpu.SemaphoreType.DMA((3 + len(_BOUNDS),)),
            pltpu.SemaphoreType.DMA((1,)),
        ],
        compiler_params=pltpu.CompilerParams(
            vmem_limit_bytes=64 * 1024 * 1024,
            disable_semaphore_checks=True,
        ),
    )(jnp.transpose(x.reshape(S, D)), w_r, w_gate, w_up, jnp.transpose(w_down))
    return jnp.transpose(out_t).reshape(B, S, D)
```

```python
import jax
import jax.numpy as jnp
from jax import lax
import jax.experimental.pallas as pl
import jax.experimental.pallas.tpu as pltpu

_C = 8
_LANES = 128
_NT = (((1,), (1,)), ((), ()))
_TN = (((0,), (0,)), ((), ()))
_INT_MIN = -(2**31)
_BOUNDS = (0, 80, 208, 320, 400, 464, 528, 576)
_CUE_ROWS, _CUE_COLS = 16, 3456
_EARLY_STRIPS = 6


def _bf16_round(v):
    return v.astype(jnp.bfloat16).astype(jnp.float32)


def _sigmoid_bf16(v):
    return _bf16_round(1.0 / _bf16_round(1.0 + _bf16_round(jnp.exp(-v))))


def _kernel(x_hbm, wr_hbm, wg_hbm, wu_hbm, wd_hbm, o_hbm,
            xb, wrb, gb, ub, db, ob, rsem, wsem):
    D, S = xb.shape
    F = db.shape[1]
    chunks = list(zip(_BOUNDS[:-1], _BOUNDS[1:]))
    r1, r2 = _BOUNDS[-3], _BOUNDS[-2]
    n_strips = S // _LANES
    strips = [i + j for j in range(4) for i in range(0, n_strips, 4)]
    early, late = strips[:_EARLY_STRIPS], strips[_EARLY_STRIPS:]
    assert len(late) >= len(early)

    c_x = pltpu.make_async_copy(x_hbm, xb, rsem.at[0])
    c_wr = pltpu.make_async_copy(wr_hbm, wrb, rsem.at[1])
    c_g = pltpu.make_async_copy(wg_hbm, gb, rsem.at[2])
    c_u = pltpu.make_async_copy(wu_hbm, ub, rsem.at[3])

    def read_d(lo, hi, c0, c1, k):
        sl = (pl.ds(lo, hi - lo), pl.ds(c0, c1 - c0))
        return pltpu.make_async_copy(wd_hbm.at[sl], db.at[sl], rsem.at[4 + k])

    n = len(chunks)
    c_d = [[read_d(lo, hi, 0, F, i)] for i, (lo, hi) in enumerate(chunks[:-1])]
    c_d[-1].append(read_d(r2, r2 + _CUE_ROWS, 0, _CUE_COLS, n - 2))
    c_d.append([read_d(r2, r2 + _CUE_ROWS, _CUE_COLS, F, n - 1),
                read_d(r2 + _CUE_ROWS, D, 0, F, n - 1)])
    for c in (c_x, c_wr, c_g, c_u, *[c for cs in c_d for c in cs]):
        c.start()

    def write(lo, hi, j):
        sl = (pl.ds(lo, hi - lo), pl.ds(j * _LANES, _LANES))
        pltpu.make_async_copy(ob.at[sl], o_hbm.at[sl], wsem.at[0]).start()

    c_x.wait()
    c_wr.wait()
    xT = xb[...]
    wr8 = jnp.broadcast_to(wrb[...].reshape(1, D), (_C, D))
    r = _bf16_round(jnp.dot(wr8, xT, preferred_element_type=jnp.float32))

    bits = pltpu.bitcast(jnp.where(r == 0.0, 0.0, r), jnp.int32)
    mono = jnp.where(bits >= 0, bits, bits ^ 0x7FFFFFFF)
    mono = jnp.where(r != r, _INT_MIN, mono & -65536)
    lane = lax.broadcasted_iota(jnp.int32, (_C, S), 1)
    row = lax.broadcasted_iota(jnp.int32, (_C, S), 0)
    key = mono | (65535 - lane)
    sel = jnp.zeros((_C, S), jnp.float32)
    for c in range(_C):
        hit = key == jnp.max(key, axis=1, keepdims=True)
        sel = jnp.where(hit & (row == c), 1.0, sel)
        key = jnp.where(hit, _INT_MIN, key)
    onehot = sel.astype(jnp.bfloat16)
    r_sel = jnp.sum(jnp.where(sel > 0, r, 0.0), axis=1, keepdims=True)
    gate = _sigmoid_bf16(r_sel)

    x_sel = lax.dot_general(onehot, xT, _NT,
                            preferred_element_type=jnp.float32).astype(jnp.bfloat16)
    c_g.wait()
    g = _bf16_round(jnp.dot(x_sel, gb[...], preferred_element_type=jnp.float32))
    g = _bf16_round(g * _sigmoid_bf16(g))
    c_u.wait()
    u = _bf16_round(jnp.dot(x_sel, ub[...], preferred_element_type=jnp.float32))
    h = (g * u).astype(jnp.bfloat16)

    for i, (lo, hi) in enumerate(chunks):
        for c in c_d[i]:
            c.wait()
        if lo == r1:
            for j in early:
                write(0, r1, j)
        y = _bf16_round(lax.dot_general(h, db[lo:hi, :], _NT,
                                        preferred_element_type=jnp.float32))
        y = (y * gate).astype(jnp.bfloat16)
        upd = lax.dot_general(y, onehot, _TN, preferred_element_type=jnp.float32)
        xc = xb[lo:hi, :].astype(jnp.float32)
        ob[lo:hi, :] = (xc + (xc * 0.0 + upd)).astype(ob.dtype)
        if lo == r1:
            for t, j in enumerate(late):
                write(0, r2, j)
                if t < len(early):
                    write(r1, r2, early[t])
    for j in strips:
        write(r2, D, j)
    pltpu.make_async_copy(ob, o_hbm, wsem.at[0]).wait()


@jax.jit
def pallas_standalone__moe_arch_mod__prompt_kernel(
    x: jax.Array,
    w_r: jax.Array,
    w_gate: jax.Array,
    w_up: jax.Array,
    w_down: jax.Array,
):
    B, S, D = x.shape
    F = w_gate.shape[1]
    assert B == 1 and D == _BOUNDS[-1] and S % (4 * _LANES) == 0
    dt = x.dtype
    params = dict(vmem_limit_bytes=64 * 1024 * 1024)
    if hasattr(pltpu.CompilerParams, "disable_semaphore_checks"):
        params["disable_semaphore_checks"] = True
    out_t = pl.pallas_call(
        _kernel,
        out_shape=jax.ShapeDtypeStruct((D, S), dt),
        in_specs=[pl.BlockSpec(memory_space=pl.ANY)] * 5,
        out_specs=pl.BlockSpec(memory_space=pl.ANY),
        scratch_shapes=[
            pltpu.VMEM((D, S), dt),
            pltpu.VMEM((D,), dt),
            pltpu.VMEM((D, F), dt),
            pltpu.VMEM((D, F), dt),
            pltpu.VMEM((D, F), dt),
            pltpu.VMEM((D, S), dt),
            pltpu.SemaphoreType.DMA((3 + len(_BOUNDS),)),
            pltpu.SemaphoreType.DMA((1,)),
        ],
        compiler_params=pltpu.CompilerParams(**params),
    )(jnp.transpose(x.reshape(S, D)), w_r, w_gate, w_up, jnp.transpose(w_down))
    return jnp.transpose(out_t).reshape(B, S, D)
```
